```python
import os as _os
_os.environ.setdefault("JAX_PLATFORMS", "cpu")
import jax
import jax.numpy as jnp

def _softmax(x, axis=-1):
    return jax.nn.softmax(x, axis=axis)
def _gelu(x):
    return jax.nn.gelu(x, approximate=True)
def _silu(x):
    return jax.nn.silu(x)
def _sigmoid(x):
    return jax.nn.sigmoid(x)
def _layernorm(x, axis=-1, eps=1e-5):
    m = jnp.mean(x, axis=axis, keepdims=True)
    v = jnp.var(x, axis=axis, keepdims=True)
    return (x - m) / jnp.sqrt(v + eps)
def _scatter_add(tgt, idx, src, axis=0):
    return tgt.at[idx].add(src)
def _segment_sum(src, seg, n):
    return jax.ops.segment_sum(src, seg, n)
class _Rng:
    def __init__(self, key):
        self._k = key
    def _next(self):
        self._k, sub = jax.random.split(self._k)
        return sub
    def normal(self, shape):
        return jax.random.normal(self._next(), shape, dtype=jnp.bfloat16)
    def randint(self, lo, hi, shape):
        return jax.random.randint(self._next(), shape, lo, hi, dtype=jnp.int32)
    def uniform(self, shape, lo=0.0, hi=1.0):
        return jax.random.uniform(self._next(), shape, jnp.bfloat16, lo, hi)
    def permutation(self, n):
        return jax.random.permutation(self._next(), n)


kernel_name = 'standalone__gqa_block_cached__near_ridge'

def setup_inputs():
    _rng = _Rng(jax.random.key(int.from_bytes(__import__("os").urandom(4), "little")))
    _w = (lambda a: (lambda t: t.astype(jnp.bfloat16) if jnp.issubdtype(t.dtype, jnp.floating) else t)(jnp.asarray(a)))
    B, Sq, D = 8, 96, 640
    Hq, Hkv, Sk, Dh = 32, 32, 512, 128
    assert Hq % Hkv == 0, (Hq, Hkv)
    return {
        "x": _w((lambda *s: _rng.normal(s) * 0.2)(B, Sq, D)),
        "k_cache": _w((lambda *s: _rng.normal(s) * 3.2)(B, Hkv, Sk, Dh)),
        "v_cache": _w((lambda *s: _rng.normal(s) * 0.05)(B, Hkv, Sk, Dh)),
        "wq": _w((lambda *s: _rng.normal(s) * 0.2)(D, Hq * Dh) * (D ** -0.5)),
        "wo": _w((lambda *s: _rng.normal(s) * 0.05)(Hq * Dh, D) * ((Hq * Dh) ** -0.5)),
    }

def reference(x, k_cache, v_cache, wq, wo):
    B, Sq, D = x.shape
    Hq, Dh = 32, 128
    Hkv = k_cache.shape[1]
    rep = Hq // Hkv
    q = (lambda x, *d: x.transpose(*d))((x @ wq).reshape(B, Sq, Hq, Dh), 0, 2, 1, 3)
    k = jnp.repeat(k_cache, rep, axis=1)
    v = jnp.repeat(v_cache, rep, axis=1)
    scores = jnp.einsum("bhqd,bhkd->bhqk", q, k) * (Dh ** -0.5)
    p = _softmax(scores, axis=-1)
    o = jnp.einsum("bhqk,bhkd->bhqd", p, v)
    return (lambda x, *d: x.transpose(*d))(o, 0, 2, 1, 3).reshape(B, Sq, Hq * Dh) @ wo
```

```python
import functools
import jax, jax.numpy as jnp, numpy as np
import jax.experimental.pallas as pl
import jax.experimental.pallas.tpu as pltpu

LOG2E = 1.4426950408889634
G = 4
NQ = 6
AHEAD = NQ - 1
NW = 4
LQ = 3
ORDER = "AECD"
CH = 128
NODMA = False
bf, f32, u32 = jnp.bfloat16, jnp.float32, jnp.uint32

def _kernel(x_hbm, k_hbm, v_hbm, wq_hbm, wo_hbm, out_hbm,
            x_v, wq_v, wo_v, k_v, v_v, q_b, s_b, p_b, l_b, o_b, acc, out_v,
            sem_x, sem_wq, sem_wo, sem_k, sem_v, sem_o,
            *, B, Sq, D, H, Sk, Dh, scale):
    NI = H * B // G
    GPH = B // G
    NC = D // 128
    NS = Sk // 128
    R = Sq // 2
    NT = Sk // CH

    kv_list = []
    for w in range(2):
        for t2 in range(NT // 2):
            for j in range(G):
                kv_list.append((w, j, 2 * t2, 0)); kv_list.append((w, j, 2 * t2 + 1, 1))

    def kv_issue(g, sel):
        slot = g % NQ
        h = g // GPH
        b0 = (g % GPH) * G
        for (w, j, t, p) in sel:
            src, dst, sem = ((k_hbm, k_v, sem_k), (v_hbm, v_v, sem_v))[w]
            pltpu.make_async_copy(src.at[b0 + j, h, pl.ds(t * CH, CH)], dst.at[slot, j, pl.ds(t * CH, CH)],
                                  sem.at[slot]).start(priority=p)
    def kv_wait(g):
        slot = g % NQ
        pltpu.make_async_copy(k_v.at[slot], k_v.at[slot], sem_k.at[slot]).wait()
        pltpu.make_async_copy(v_v.at[slot], v_v.at[slot], sem_v.at[slot]).wait()
    def wq_issue(h, sel):
        slot = h % NW
        for c in sel:
            pltpu.make_async_copy(wq_hbm.at[pl.ds(c * 128, 128), pl.ds(pl.multiple_of(h * Dh, Dh), Dh)],
                                  wq_v.at[slot, pl.ds(c * 128, 128)], sem_wq.at[slot]).start(priority=c % 2)
    def wq_wait(h):
        slot = h % NW
        pltpu.make_async_copy(wq_v.at[slot], wq_v.at[slot], sem_wq.at[slot]).wait()
    def wo_issue(h, sel):
        slot = h % NW
        for c in sel:
            pltpu.make_async_copy(wo_hbm.at[pl.ds(pl.multiple_of(h * Dh, Dh), Dh), pl.ds(c * 128, 128)],
                                  wo_v.at[slot, c], sem_wo.at[slot]).start(priority=(c + 1) % 2)
    def wo_wait(h):
        slot = h % NW
        pltpu.make_async_copy(wo_v.at[slot], wo_v.at[slot], sem_wo.at[slot]).wait()
    def w_issue(g, sel, static=False):
        if static:
            if g % 2 == 0: wo_issue(g // 2, sel)
            elif (g + 1) // 2 < H: wq_issue((g + 1) // 2, sel)
        else:
            pl.when(jnp.logical_and(g < NI, g % 2 == 0))(lambda: wo_issue(g // 2, sel))
            pl.when(jnp.logical_and(g < NI - 1, g % 2 == 1))(lambda: wq_issue((g + 1) // 2, sel))
    def w_wait(g):
        pl.when(g % 2 == 0)(lambda: wo_wait(g // 2))
        pl.when(jnp.logical_and(g < NI - 1, g % 2 == 1))(lambda: wq_wait((g + 1) // 2))
    def out_issue(b):
        rows = pl.ds(pl.multiple_of(b * Sq, Sq), Sq)
        pltpu.make_async_copy(out_v.at[rows], out_hbm.at[rows], sem_o).start()

    x_u, wq_u, wo_u, k_u, v_u = (r.bitcast(u32) for r in (x_v, wq_v, wo_v, k_v, v_v))
    q_u, p_u, o_u = (r.bitcast(u32) for r in (q_b, p_b, o_b))
    def ldbf(v):
        return pltpu.bitcast(v, bf)
    def stage_E(t, js):
        tc = jnp.minimum(t, H * B - 1)
        h = tc // B; b = tc % B
        rows = pl.ds(pl.multiple_of(b * R, R), R)
        xb = jnp.concatenate([ldbf(x_u[c, rows, :]) for c in range(NC)], axis=1)
        q = jnp.dot(xb, ldbf(wq_u[h % NW]), preferred_element_type=f32)
        q_b[js % 4] = q.astype(bf)
    def stage_A(g, j):
        q = ldbf(q_u[j])
        k = ldbf(k_u[g % NQ, j])
        s_b[j % 2] = jax.lax.dot_general(q, k, (((1,), (1,)), ((), ())), preferred_element_type=f32)
    def stage_B(j):
        s = s_b[j % 2]
        m = jnp.max(s, axis=-1, keepdims=True)
        p = jnp.exp2((s - m) * (scale * LOG2E))
        l = jnp.sum(p, axis=-1, keepdims=True)
        pb = p.astype(bf)
        for c in range(NS):
            p_b[j % 2, c] = pb[:, c * 128:(c + 1) * 128]
        lb = jnp.broadcast_to(l, (Sq, Dh))
        r = pl.reciprocal(lb, approx=True)
        l_b[j % 2] = r * (2.0 - lb * r)
    def stage_C(g, j, js):
        v = ldbf(v_u[g % NQ, j])
        p = jnp.concatenate([ldbf(p_u[js % 2, c]) for c in range(NS)], axis=1)
        o = jnp.dot(p, v, preferred_element_type=f32)
        o = o * l_b[js % 2]
        o_b[js % 2] = o.astype(bf)
    def stage_D(t, js):
        tc = jnp.maximum(t, 0)
        h = tc // B
        b = jnp.where(t < 0, B, tc % B)
        w = jnp.concatenate([ldbf(wo_u[h % NW, c]) for c in range(NC)], axis=1)
        r = jnp.dot(ldbf(o_u[js % 2]), w, preferred_element_type=f32)
        rows = pl.ds(pl.multiple_of(b * Sq, Sq), Sq)
        a = acc[rows, :] + r
        acc[rows, :] = a
        out_v[rows, :] = a.astype(bf)
        if isinstance(t, int):
            if t >= (H - 1) * B: out_issue(t % B)
        else:
            pl.when(t >= (H - 1) * B)(lambda: out_issue(b))

    for b in range(B):
        for c in range(NC):
            pltpu.make_async_copy(x_hbm.at[pl.ds(b * Sq, Sq), pl.ds(c * 128, 128)], x_v.at[c, pl.ds(b * Sq, Sq)], sem_x).start(priority=c % 2)
        if b == G - 1:
            wq_issue(0, range(NC))
            kv_issue(0, kv_list)
            w_issue(0, range(NC), True)
    for g in range(1, AHEAD):
        kv_issue(g, kv_list)
        w_issue(g, range(NC), True)
    if NODMA:
        for g in range(AHEAD):
            kv_wait(g)
            if g % 2 == 0: wo_wait(g // 2)
            else: wq_wait((g + 1) // 2)
    acc[...] = jnp.zeros_like(acc)
    pltpu.make_async_copy(x_v, x_v, sem_x).wait()
    wq_wait(0)
    for b in range(LQ):
        stage_E(b, b)

    nkv = len(kv_list) // G
    wsel = [[0, 1], [2], [3], [4]]
    def body(i, c):
        if not NODMA:
            kv_wait(i)
            w_wait(i)
        gi = i + AHEAD
        for j in range(G):
            t = i * G + j
            for q in range(0, nkv, 4):
                sel = kv_list[j * nkv + q: j * nkv + q + 4]
                if not NODMA: pl.when(gi < NI)(functools.partial(kv_issue, gi, sel))
            if not NODMA: w_issue(gi, wsel[j])
            for st in ORDER:
                if st == 'A':
                    stage_A(i, j); stage_B(j)
                elif st == 'E':
                    stage_E(t + LQ, j + LQ)
                elif st == 'C':
                    if j == 0:
                        stage_C(jnp.maximum(i - 1, 0), G - 1, j - 1)
                    else:
                        stage_C(i, j - 1, j - 1)
                elif st == 'D':
                    stage_D(t - 2, j - 2)
        return c
    jax.lax.fori_loop(0, NI, body, 0)
    T = H * B
    stage_C(NI - 1, G - 1, G - 1)
    stage_D(T - 2, G - 2)
    stage_D(T - 1, G - 1)
    pltpu.make_async_copy(out_v.at[pl.ds(0, B * Sq)], out_hbm, sem_o).wait()


@jax.jit
def pallas_standalone__gqa_block_cached__near_ridge_kernel(x, k_cache, v_cache, wq, wo):
    B, Sq, D = x.shape
    _, H, Sk, Dh = k_cache.shape
    x2 = x.reshape(B * Sq, D)
    NC = D // 128
    out = pl.pallas_call(
        functools.partial(_kernel, B=B, Sq=Sq, D=D, H=H, Sk=Sk, Dh=Dh, scale=Dh ** -0.5),
        in_specs=[pl.BlockSpec(memory_space=pl.ANY)] * 5,
        out_specs=pl.BlockSpec(memory_space=pl.ANY),
        out_shape=jax.ShapeDtypeStruct((B * Sq, D), x.dtype),
        scratch_shapes=[
            pltpu.VMEM((NC, B * Sq, 128), bf), pltpu.VMEM((NW, D, Dh), bf), pltpu.VMEM((NW, NC, Dh, 128), bf),
            pltpu.VMEM((NQ, G, Sk, Dh), bf), pltpu.VMEM((NQ, G, Sk, Dh), bf),
            pltpu.VMEM((4, Sq, Dh), bf), pltpu.VMEM((2, Sq, Sk), f32), pltpu.VMEM((2, Sk // 128, Sq, 128), bf),
            pltpu.VMEM((2, Sq, Dh), f32), pltpu.VMEM((2, Sq, Dh), bf),
            pltpu.VMEM(((B + 1) * Sq, D), f32), pltpu.VMEM(((B + 1) * Sq, D), bf),
            pltpu.SemaphoreType.DMA, pltpu.SemaphoreType.DMA((NW,)), pltpu.SemaphoreType.DMA((NW,)),
            pltpu.SemaphoreType.DMA((NQ,)), pltpu.SemaphoreType.DMA((NQ,)), pltpu.SemaphoreType.DMA,
        ],
        compiler_params=pltpu.CompilerParams(vmem_limit_bytes=100 * 1024 * 1024, disable_bounds_checks=True),
    )(x2, k_cache, v_cache, wq, wo)
    return out.reshape(B, Sq, D)
```

```python
import functools

import jax
import jax.numpy as jnp
import jax.experimental.pallas as pl
import jax.experimental.pallas.tpu as pltpu

LOG2E = 1.4426950408889634
G = 2
LEAD = (3, 5)
NQ = 8
NW = 4
LQ = 3
LAG = 2
CH = 128


def _kernel(x_hbm, k_hbm, v_hbm, wq_hbm, wo_hbm, out_hbm,
            x_v, wq_v, wo_v, k_v, v_v, q_b, s_b, p_b, l_b, o_b, acc, out_v, sz_v,
            sem_x, sem_w0, sem_u, sem_o,
            *, B, Sq, D, H, Sk, Dh, scale):
    bf, f32, u32 = jnp.bfloat16, jnp.float32, jnp.uint32
    NI = H * B // G
    UPH = B // G
    NC = D // 128
    NS = Sk // 128
    R = Sq // 2
    NT = Sk // CH
    T = H * B
    HALF = UPH // 2
    WR_Q = D // UPH
    WR_O = Dh // UPH
    NOW = NI - 3

    def when(pred, fn):
        if isinstance(pred, bool):
            if pred:
                fn()
        else:
            pl.when(pred)(fn)

    def mult(i, n):
        return i if isinstance(i, int) else pl.multiple_of(i, n)

    kv_list = []
    for t2 in range(NT // 2):
        for w in range(2):
            for j in range(G):
                kv_list.append((w, j, 2 * t2, 0))
                kv_list.append((w, j, 2 * t2 + 1, 1))

    def kv_issue(u, e, prio=None):
        w, j, t, p = e
        src, dst = ((k_hbm, k_v), (v_hbm, v_v))[w]
        slot = u % NQ
        pltpu.make_async_copy(src.at[(u % UPH) * G + j, u // UPH, pl.ds(t * CH, CH)],
                              dst.at[slot, j, pl.ds(t * CH, CH)],
                              sem_u.at[slot]).start(priority=p if prio is None else prio)

    def wq_copy(h, piece, sem):
        rows = pl.ds(mult(piece * WR_Q, WR_Q), WR_Q)
        return pltpu.make_async_copy(wq_hbm.at[rows, pl.ds(mult(h * Dh, Dh), Dh)],
                                     wq_v.at[h % NW, rows], sem)

    def wo_copy(h, piece, sem):
        r0 = piece * WR_O
        return pltpu.make_async_copy(wo_hbm.at[pl.ds(mult(h * Dh + r0, WR_O), WR_O)],
                                     wo_v.at[h % NW, pl.ds(mult(r0, WR_O), WR_O)], sem)

    def w_issue(u, p, prio=None):
        prio = p if prio is None else prio
        hh = (u + 1) // UPH
        ph = (u + 1) % UPH
        sem = sem_u.at[u % NQ]
        if isinstance(u, int):
            if ph < HALF and hh < H:
                wo_copy(hh, 2 * ph + p, sem).start(priority=prio)
            elif ph >= HALF and hh + 1 < H:
                wq_copy(hh + 1, 2 * (ph - HALF) + p, sem).start(priority=prio)
        else:
            pl.when(jnp.logical_and(ph < HALF, hh < H))(
                lambda: wo_copy(hh, 2 * ph + p, sem).start(priority=prio))
            pl.when(jnp.logical_and(ph >= HALF, hh + 1 < H))(
                lambda: wq_copy(hh + 1, 2 * (ph - HALF) + p, sem).start(priority=prio))

    def unit_wait(u):
        sem = sem_u.at[u % NQ]
        szk = sz_v.at[pl.ds(0, 2 * G * Sk)]
        when(u < NOW, lambda: pltpu.make_async_copy(sz_v, sz_v, sem).wait())
        when(u >= NOW, lambda: pltpu.make_async_copy(szk, szk, sem).wait())

    def out_issue(b):
        rows = pl.ds(b * Sq, Sq)
        pltpu.make_async_copy(out_v.at[rows], out_hbm.at[rows], sem_o).start()

    stages = "AECD"
    npos = G * len(stages)
    q_lists = []
    for p in range(2):
        l = [e for e in kv_list if e[3] == p]
        l.insert(len(l) // 2, "w")
        q_lists.append(l)
    sched = [[] for _ in range(npos + LAG)]
    for p in range(2):
        for n, e in enumerate(q_lists[p]):
            pos = 0 if n == 0 else LAG + ((n - 1) * npos) // (len(q_lists[p]) - 1)
            sched[pos].append((p, e))

    x_u, wq_u, k_u, v_u, q_u, p_u, o_u = (
        r.bitcast(u32) for r in (x_v, wq_v, k_v, v_v, q_b, p_b, o_b))

    def ldbf(v):
        return pltpu.bitcast(v, bf)

    def stage_E(t, qs):
        h, b = t // B, t % B
        rows = pl.ds(mult(b * R, R), R)
        xb = jnp.concatenate([ldbf(x_u[c, rows, :]) for c in range(NC)], axis=1)
        qb = jnp.dot(xb, ldbf(wq_u[h % NW]), preferred_element_type=f32).astype(bf)
        q_b[qs] = qb
        return qb[0:16, :]

    def stage_A(u, j, qs):
        s = jax.lax.dot_general(ldbf(q_u[qs]), ldbf(k_u[u % NQ, j]), (((1,), (1,)), ((), ())),
                                preferred_element_type=f32)
        s_b[j % 2] = s
        return s[0:16, 0:128].astype(bf)

    def stage_B(j):
        s = s_b[j % 2]
        m = jnp.max(s, axis=-1, keepdims=True)
        p = jnp.exp2((s - m) * (scale * LOG2E))
        l = jnp.sum(p, axis=-1, keepdims=True)
        pb = p.astype(bf)
        for c in range(NS):
            p_b[j % 2, c] = pb[:, c * 128:(c + 1) * 128]
        lb = jnp.broadcast_to(l, (Sq, Dh))
        r = pl.reciprocal(lb, approx=True)
        l_b[j % 2] = r * (2.0 - lb * r)

    def stage_C(u, j, js):
        p = jnp.concatenate([ldbf(p_u[js % 2, c]) for c in range(NS)], axis=1)
        o = jnp.dot(p, ldbf(v_u[u % NQ, j]), preferred_element_type=f32)
        ob = (o * l_b[js % 2]).astype(bf)
        o_b[js % 2] = ob
        return ob[0:16, :]

    def stage_D(t, js):
        if isinstance(t, int):
            h, b = t // B, t % B
            rows = pl.ds(b * Sq, Sq)
        else:
            tc = jnp.maximum(t, 0)
            h = tc // B
            b = jnp.where(t < 0, B, tc % B)
            rows = pl.ds(pl.multiple_of(b * Sq, Sq), Sq)
        a = acc[rows, :] + jnp.dot(ldbf(o_u[js % 2]), wo_v[h % NW], preferred_element_type=f32)
        if isinstance(t, int) and t >= (H - 1) * B:
            out_v[rows, :] = a.astype(bf)
            out_issue(b)
        else:
            acc[rows, :] = a
        return a[0:16, 0:128].astype(bf)

    def x_issue(b, prio):
        for c in range(NC):
            pltpu.make_async_copy(x_hbm.at[pl.ds(b * Sq, Sq), pl.ds(c * 128, 128)],
                                  x_v.at[c, pl.ds(b * Sq, Sq)],
                                  sem_x.at[0 if b < LQ else 1]).start(priority=prio)

    def unit_issue_static(u):
        for p in range(2):
            if u < LEAD[p]:
                for e in q_lists[p]:
                    if e == "w":
                        w_issue(u, p, 1)
                    else:
                        kv_issue(u, e, 1)

    for piece in range(UPH):
        wq_copy(0, piece, sem_w0).start(priority=0)
    for b in range(LQ):
        x_issue(b, 0)
    for piece in range(2):
        wo_copy(0, piece, sem_x.at[1]).start(priority=1)
    pl.delay(1)
    unit_issue_static(0)
    for b in range(LQ, B):
        x_issue(b, 1)
    pl.delay(1)
    for u in range(1, max(LEAD)):
        unit_issue_static(u)
        pl.delay(1)
    acc[...] = jnp.zeros_like(acc)
    p_b[...] = jnp.zeros_like(p_b)
    l_b[...] = jnp.zeros_like(l_b)
    o_b[...] = jnp.zeros_like(o_b)
    pltpu.make_async_copy(x_v.at[:, pl.ds(0, LQ * Sq)], x_v.at[:, pl.ds(0, LQ * Sq)], sem_x.at[0]).wait()
    pltpu.make_async_copy(wq_v.at[0], wq_v.at[0], sem_w0).wait()
    for t in range(LQ):
        stage_E(t, t)
    pltpu.make_async_copy(x_v.at[:, pl.ds(0, (B - LQ) * Sq)], x_v.at[:, pl.ds(0, (B - LQ) * Sq)],
                          sem_x.at[1]).wait()
    wsz = wq_v.at[0, pl.ds(0, 2 * WR_Q)]
    pltpu.make_async_copy(wsz, wsz, sem_x.at[1]).wait()

    def unit(u, k):
        unit_wait(u)
        pins = []

        def point(pos):
            es = sched[pos]
            if pos >= LAG:
                pv = pins[pos - LAG]
                for w in sorted(set("w" if e == "w" else "kv"[e[0]] for _, e in es)):
                    if w == "w":
                        wq_v[NW, 0:16, :] = pv
                        wo_v[NW, 0:16, 0:128] = pv
                    else:
                        (k_v if w == "k" else v_v)[NQ, 0, 0:16, :] = pv
            for p, e in es:
                uu = u + LEAD[p]
                if e == "w":
                    w_issue(uu, p)
                else:
                    pl.when(uu < NI)(functools.partial(kv_issue, uu, e))

        for j in range(G):
            t = u * G + j
            for st in stages:
                if st == "A":
                    r = stage_A(u, j, (k * G + j) % 4)
                    stage_B(j)
                elif st == "E":
                    r = stage_E(t + LQ, (k * G + j + LQ) % 4)
                elif st == "C":
                    if j == 0:
                        r = stage_C(jnp.maximum(u - 1, 0), G - 1, j - 1)
                    else:
                        r = stage_C(u, j - 1, j - 1)
                else:
                    r = stage_D(t - 2, j - 2)
                pins.append(r)
                point(len(pins) - 1)
        for pos in range(npos, npos + LAG):
            point(pos)

    def body(i, carry):
        unit(2 * i, 0)
        unit(2 * i + 1, 1)
        return carry

    jax.lax.fori_loop(0, (NI - 2) // 2, body, 0)

    u0, u1 = NI - 2, NI - 1
    t0 = u0 * G
    unit_wait(u0)
    unit_wait(u1)
    stage_A(u0, 0, 0)
    stage_B(0)
    for tb in range((H - 1) * B, t0 - 2):
        rows = pl.ds((tb % B) * Sq, Sq)
        out_v[rows, :] = acc[rows, :].astype(bf)
        out_issue(tb % B)
    for te in range(t0 + LQ, T):
        stage_E(te, te % 4)
    stage_C(u0 - 1, 1, 1)
    stage_D(t0 - 2, 0)
    stage_A(u0, 1, 1)
    stage_B(1)
    stage_C(u0, 0, 0)
    stage_D(t0 - 1, 1)
    stage_A(u1, 0, 2)
    stage_B(0)
    stage_C(u0, 1, 1)
    stage_A(u1, 1, 3)
    stage_B(1)
    stage_D(t0, 0)
    stage_C(u1, 0, 0)
    stage_D(t0 + 1, 1)
    stage_C(u1, 1, 1)
    stage_D(t0 + 2, 0)
    stage_D(t0 + 3, 1)
    pltpu.make_async_copy(out_v.at[pl.ds(0, B * Sq)], out_hbm, sem_o).wait()


@jax.jit
def pallas_standalone__gqa_block_cached__near_ridge_kernel(
    x: jax.Array,
    k_cache: jax.Array,
    v_cache: jax.Array,
    wq: jax.Array,
    wo: jax.Array,
):
    B, Sq, D = x.shape
    _, H, Sk, Dh = k_cache.shape
    assert wq.shape == (D, H * Dh) and wo.shape == (H * Dh, D)
    assert (B, Sq, D, H, Sk, Dh) == (8, 96, 640, 32, 512, 128)
    bf, f32 = jnp.bfloat16, jnp.float32
    UPH = B // G
    out = pl.pallas_call(
        functools.partial(_kernel, B=B, Sq=Sq, D=D, H=H, Sk=Sk, Dh=Dh, scale=Dh ** -0.5),
        in_specs=[pl.BlockSpec(memory_space=pl.ANY)] * 5,
        out_specs=pl.BlockSpec(memory_space=pl.ANY),
        out_shape=jax.ShapeDtypeStruct((B * Sq, D), x.dtype),
        scratch_shapes=[
            pltpu.VMEM((D // 128, B * Sq, 128), bf),
            pltpu.VMEM((NW + 1, D, Dh), bf),
            pltpu.VMEM((NW + 1, Dh, D), bf),
            pltpu.VMEM((NQ + 1, G, Sk, Dh), bf),
            pltpu.VMEM((NQ + 1, G, Sk, Dh), bf),
            pltpu.VMEM((4, Sq, Dh), bf),
            pltpu.VMEM((2, Sq, Sk), f32),
            pltpu.VMEM((2, Sk // 128, Sq, 128), bf),
            pltpu.VMEM((2, Sq, Dh), f32),
            pltpu.VMEM((2, Sq, Dh), bf),
            pltpu.VMEM(((B + 1) * Sq, D), f32),
            pltpu.VMEM((B * Sq, D), bf),
            pltpu.VMEM((2 * G * Sk + 2 * (D // UPH), Dh), bf),
            pltpu.SemaphoreType.DMA((2,)),
            pltpu.SemaphoreType.DMA,
            pltpu.SemaphoreType.DMA((NQ,)),
            pltpu.SemaphoreType.DMA,
        ],
        compiler_params=pltpu.CompilerParams(
            vmem_limit_bytes=64 * 1024 * 1024,
            disable_bounds_checks=True,
            disable_semaphore_checks=True,
        ),
    )(x.reshape(B * Sq, D), k_cache, v_cache, wq, wo)
    return out.reshape(B, Sq, D)
```

```python
import functools

import jax
import jax.numpy as jnp
import jax.experimental.pallas as pl
import jax.experimental.pallas.tpu as pltpu

LOG2E = 1.4426950408889634
G = 2
LEAD = (3, 5)
NQ = 8
NW = 4
LQ = 3
LAG = 3
TAPER = 112
CH = 128


def _kernel(x_hbm, k_hbm, v_hbm, wq_hbm, wo_hbm, out_hbm,
            x_v, wq_v, wo_v, k_v, v_v, q_b, s_b, p_b, l_b, o_b, acc, out_v, sz_v,
            sem_x, sem_w0, sem_u, sem_o,
            *, B, Sq, D, H, Sk, Dh, scale):
    bf, f32, u32 = jnp.bfloat16, jnp.float32, jnp.uint32
    NI = H * B // G
    UPH = B // G
    NC = D // 128
    NS = Sk // 128
    R = Sq // 2
    NT = Sk // CH
    T = H * B
    HALF = UPH // 2
    WR_Q = D // UPH
    WR_O = Dh // UPH
    NOW = NI - 3

    def when(pred, fn):
        if isinstance(pred, bool):
            if pred:
                fn()
        else:
            pl.when(pred)(fn)

    def mult(i, n):
        return i if isinstance(i, int) else pl.multiple_of(i, n)

    kv_list = []
    for t2 in range(NT // 2):
        for w in range(2):
            for j in range(G):
                kv_list.append((w, j, 2 * t2, 0))
                kv_list.append((w, j, 2 * t2 + 1, 1))

    def kv_issue(u, e, prio=None):
        w, j, t, p = e
        src, dst = ((k_hbm, k_v), (v_hbm, v_v))[w]
        slot = u % NQ
        pltpu.make_async_copy(src.at[(u % UPH) * G + j, u // UPH, pl.ds(t * CH, CH)],
                              dst.at[slot, j, pl.ds(t * CH, CH)],
                              sem_u.at[slot]).start(priority=p if prio is None else prio)

    def wq_copy(h, piece, sem):
        rows = pl.ds(mult(piece * WR_Q, WR_Q), WR_Q)
        return pltpu.make_async_copy(wq_hbm.at[rows, pl.ds(mult(h * Dh, Dh), Dh)],
                                     wq_v.at[h % NW, rows], sem)

    def wo_copy(h, piece, sem):
        r0 = piece * WR_O
        return pltpu.make_async_copy(wo_hbm.at[pl.ds(mult(h * Dh + r0, WR_O), WR_O)],
                                     wo_v.at[h % NW, pl.ds(mult(r0, WR_O), WR_O)], sem)

    def w_issue(u, p, prio=None):
        prio = p if prio is None else prio
        hh = (u + 1) // UPH
        ph = (u + 1) % UPH
        sem = sem_u.at[u % NQ]
        if isinstance(u, int):
            if ph < HALF and hh < H:
                wo_copy(hh, 2 * ph + p, sem).start(priority=prio)
            elif ph >= HALF and hh + 1 < H:
                wq_copy(hh + 1, 2 * (ph - HALF) + p, sem).start(priority=prio)
        else:
            pl.when(jnp.logical_and(ph < HALF, hh < H))(
                lambda: wo_copy(hh, 2 * ph + p, sem).start(priority=prio))
            pl.when(jnp.logical_and(ph >= HALF, hh + 1 < H))(
                lambda: wq_copy(hh + 1, 2 * (ph - HALF) + p, sem).start(priority=prio))

    def unit_wait(u):
        sem = sem_u.at[u % NQ]
        szk = sz_v.at[pl.ds(0, 2 * G * Sk)]
        when(u < NOW, lambda: pltpu.make_async_copy(sz_v, sz_v, sem).wait())
        when(u >= NOW, lambda: pltpu.make_async_copy(szk, szk, sem).wait())

    def out_issue(b):
        rows = pl.ds(b * Sq, Sq)
        pltpu.make_async_copy(out_v.at[rows], out_hbm.at[rows], sem_o).start()

    stages = "AECD"
    npos = G * len(stages)
    q_lists = []
    for p in range(2):
        l = [e for e in kv_list if e[3] == p]
        l.insert(len(l) // 2, "w")
        q_lists.append(l)
    sched = [[] for _ in range(npos + LAG)]
    for p in range(2):
        for n, e in enumerate(q_lists[p]):
            pos = 0 if n == 0 else LAG + ((n - 1) * npos) // (len(q_lists[p]) - 1)
            sched[pos].append((p, e))

    x_u, wq_u, k_u, v_u, q_u, p_u, o_u = (
        r.bitcast(u32) for r in (x_v, wq_v, k_v, v_v, q_b, p_b, o_b))

    def ldbf(v):
        return pltpu.bitcast(v, bf)

    def stage_E(t, qs):
        h, b = t // B, t % B
        rows = pl.ds(mult(b * R, R), R)
        xb = jnp.concatenate([ldbf(x_u[c, rows, :]) for c in range(NC)], axis=1)
        qb = jnp.dot(xb, ldbf(wq_u[h % NW]), preferred_element_type=f32).astype(bf)
        q_b[qs] = qb
        return qb[0:16, :]

    def stage_A(u, j, qs):
        s = jax.lax.dot_general(ldbf(q_u[qs]), ldbf(k_u[u % NQ, j]), (((1,), (1,)), ((), ())),
                                preferred_element_type=f32)
        s_b[j % 2] = s
        return s[0:16, 0:128].astype(bf)

    def stage_B(j):
        s = s_b[j % 2]
        m = jnp.max(s, axis=-1, keepdims=True)
        p = jnp.exp2((s - m) * (scale * LOG2E))
        l = jnp.sum(p, axis=-1, keepdims=True)
        pb = p.astype(bf)
        for c in range(NS):
            p_b[j % 2, c] = pb[:, c * 128:(c + 1) * 128]
        lb = jnp.broadcast_to(l, (Sq, Dh))
        r = pl.reciprocal(lb, approx=True)
        l_b[j % 2] = r * (2.0 - lb * r)

    def stage_C(u, j, js):
        p = jnp.concatenate([ldbf(p_u[js % 2, c]) for c in range(NS)], axis=1)
        o = jnp.dot(p, ldbf(v_u[u % NQ, j]), preferred_element_type=f32)
        ob = (o * l_b[js % 2]).astype(bf)
        o_b[js % 2] = ob
        return ob[0:16, :]

    def stage_D(t, js):
        if isinstance(t, int):
            h, b = t // B, t % B
            rows = pl.ds(b * Sq, Sq)
        else:
            tc = jnp.maximum(t, 0)
            h = tc // B
            b = jnp.where(t < 0, B, tc % B)
            rows = pl.ds(pl.multiple_of(b * Sq, Sq), Sq)
        a = acc[rows, :] + jnp.dot(ldbf(o_u[js % 2]), wo_v[h % NW], preferred_element_type=f32)
        if isinstance(t, int) and t >= (H - 1) * B:
            out_v[rows, :] = a.astype(bf)
            out_issue(b)
        else:
            acc[rows, :] = a
        return a[0:16, 0:128].astype(bf)

    def x_issue(b, prio):
        for c in range(NC):
            pltpu.make_async_copy(x_hbm.at[pl.ds(b * Sq, Sq), pl.ds(c * 128, 128)],
                                  x_v.at[c, pl.ds(b * Sq, Sq)],
                                  sem_x.at[0 if b < LQ else 1]).start(priority=prio)

    def unit_issue_static(u):
        for p in range(2):
            if u < LEAD[p]:
                for e in q_lists[p]:
                    if e == "w":
                        w_issue(u, p, 1)
                    else:
                        kv_issue(u, e, 1)

    for piece in range(UPH):
        wq_copy(0, piece, sem_w0).start(priority=0)
    for b in range(LQ):
        x_issue(b, 0)
    for piece in range(2):
        wo_copy(0, piece, sem_x.at[1]).start(priority=1)
    pl.delay(1)
    unit_issue_static(0)
    for b in range(LQ, B):
        x_issue(b, 1)
    pl.delay(1)
    for u in range(1, max(LEAD)):
        unit_issue_static(u)
        pl.delay(1)
    acc[...] = jnp.zeros_like(acc)
    p_b[...] = jnp.zeros_like(p_b)
    l_b[...] = jnp.zeros_like(l_b)
    o_b[...] = jnp.zeros_like(o_b)
    pltpu.make_async_copy(x_v.at[:, pl.ds(0, LQ * Sq)], x_v.at[:, pl.ds(0, LQ * Sq)], sem_x.at[0]).wait()
    pltpu.make_async_copy(wq_v.at[0], wq_v.at[0], sem_w0).wait()
    for t in range(LQ):
        stage_E(t, t)
    pltpu.make_async_copy(x_v.at[:, pl.ds(0, (B - LQ) * Sq)], x_v.at[:, pl.ds(0, (B - LQ) * Sq)],
                          sem_x.at[1]).wait()
    wsz = wq_v.at[0, pl.ds(0, 2 * WR_Q)]
    pltpu.make_async_copy(wsz, wsz, sem_x.at[1]).wait()

    def unit(u, k):
        unit_wait(u)
        pins = []
        tgt = [jnp.where(u < TAPER, u + LEAD[0], jnp.where(u == TAPER, NI, u + LEAD[0] - 1)),
               u + LEAD[1]]

        def point(pos):
            es = sched[pos]
            if pos >= LAG:
                pv = pins[pos - LAG]
                for w in sorted(set("w" if e == "w" else "kv"[e[0]] for _, e in es)):
                    if w == "w":
                        wq_v[NW, 0:16, :] = pv
                        wo_v[NW, 0:16, 0:128] = pv
                    else:
                        (k_v if w == "k" else v_v)[NQ, 0, 0:16, :] = pv
            for p, e in es:
                uu = tgt[p]
                if e == "w":
                    w_issue(uu, p)
                else:
                    pl.when(uu < NI)(functools.partial(kv_issue, uu, e))

        for j in range(G):
            t = u * G + j
            for st in stages:
                if st == "A":
                    r = stage_A(u, j, (k * G + j) % 4)
                    stage_B(j)
                elif st == "E":
                    r = stage_E(t + LQ, (k * G + j + LQ) % 4)
                elif st == "C":
                    if j == 0:
                        r = stage_C(jnp.maximum(u - 1, 0), G - 1, j - 1)
                    else:
                        r = stage_C(u, j - 1, j - 1)
                else:
                    r = stage_D(t - 2, j - 2)
                pins.append(r)
                point(len(pins) - 1)
        for pos in range(npos, npos + LAG):
            point(pos)

    def body(i, carry):
        unit(2 * i, 0)
        unit(2 * i + 1, 1)
        return carry

    jax.lax.fori_loop(0, (NI - 2) // 2, body, 0)

    u0, u1 = NI - 2, NI - 1
    t0 = u0 * G
    unit_wait(u0)
    stage_A(u0, 0, 0)
    stage_B(0)
    for te in range(t0 + LQ, T):
        stage_E(te, te % 4)
    stage_C(u0 - 1, 1, 1)
    stage_D(t0 - 2, 0)
    stage_A(u0, 1, 1)
    stage_B(1)
    stage_C(u0, 0, 0)
    stage_D(t0 - 1, 1)
    for tb in range((H - 1) * B, t0 - 2):
        rows = pl.ds((tb % B) * Sq, Sq)
        out_v[rows, :] = acc[rows, :].astype(bf)
        out_issue(tb % B)
    unit_wait(u1)
    stage_A(u1, 0, 2)
    stage_B(0)
    stage_C(u0, 1, 1)
    stage_A(u1, 1, 3)
    stage_B(1)
    stage_D(t0, 0)
    stage_C(u1, 0, 0)
    stage_D(t0 + 1, 1)
    stage_C(u1, 1, 1)
    stage_D(t0 + 2, 0)
    stage_D(t0 + 3, 1)
    pltpu.make_async_copy(out_v.at[pl.ds(0, B * Sq)], out_hbm, sem_o).wait()


@jax.jit
def pallas_standalone__gqa_block_cached__near_ridge_kernel(
    x: jax.Array,
    k_cache: jax.Array,
    v_cache: jax.Array,
    wq: jax.Array,
    wo: jax.Array,
):
    B, Sq, D = x.shape
    _, H, Sk, Dh = k_cache.shape
    assert wq.shape == (D, H * Dh) and wo.shape == (H * Dh, D)
    assert (B, Sq, D, H, Sk, Dh) == (8, 96, 640, 32, 512, 128)
    bf, f32 = jnp.bfloat16, jnp.float32
    UPH = B // G
    out = pl.pallas_call(
        functools.partial(_kernel, B=B, Sq=Sq, D=D, H=H, Sk=Sk, Dh=Dh, scale=Dh ** -0.5),
        in_specs=[pl.BlockSpec(memory_space=pl.ANY)] * 5,
        out_specs=pl.BlockSpec(memory_space=pl.ANY),
        out_shape=jax.ShapeDtypeStruct((B * Sq, D), x.dtype),
        scratch_shapes=[
            pltpu.VMEM((D // 128, B * Sq, 128), bf),
            pltpu.VMEM((NW + 1, D, Dh), bf),
            pltpu.VMEM((NW + 1, Dh, D), bf),
            pltpu.VMEM((NQ + 1, G, Sk, Dh), bf),
            pltpu.VMEM((NQ + 1, G, Sk, Dh), bf),
            pltpu.VMEM((4, Sq, Dh), bf),
            pltpu.VMEM((2, Sq, Sk), f32),
            pltpu.VMEM((2, Sk // 128, Sq, 128), bf),
            pltpu.VMEM((2, Sq, Dh), f32),
            pltpu.VMEM((2, Sq, Dh), bf),
            pltpu.VMEM(((B + 1) * Sq, D), f32),
            pltpu.VMEM((B * Sq, D), bf),
            pltpu.VMEM((2 * G * Sk + 2 * (D // UPH), Dh), bf),
            pltpu.SemaphoreType.DMA((2,)),
            pltpu.SemaphoreType.DMA,
            pltpu.SemaphoreType.DMA((NQ,)),
            pltpu.SemaphoreType.DMA,
        ],
        compiler_params=pltpu.CompilerParams(
            vmem_limit_bytes=64 * 1024 * 1024,
            disable_bounds_checks=True,
            disable_semaphore_checks=True,
        ),
    )(x.reshape(B * Sq, D), k_cache, v_cache, wq, wo)
    return out.reshape(B, Sq, D)
```
